```python
import os as _os
_os.environ.setdefault("JAX_PLATFORMS", "cpu")
import jax
import jax.numpy as jnp

def _softmax(x, axis=-1):
    return jax.nn.softmax(x, axis=axis)
def _gelu(x):
    return jax.nn.gelu(x, approximate=True)
def _silu(x):
    return jax.nn.silu(x)
def _sigmoid(x):
    return jax.nn.sigmoid(x)
def _layernorm(x, axis=-1, eps=1e-5):
    m = jnp.mean(x, axis=axis, keepdims=True)
    v = jnp.var(x, axis=axis, keepdims=True)
    return (x - m) / jnp.sqrt(v + eps)
def _scatter_add(tgt, idx, src, axis=0):
    return tgt.at[idx].add(src)
def _segment_sum(src, seg, n):
    return jax.ops.segment_sum(src, seg, n)
class _Rng:
    def __init__(self, key):
        self._k = key
    def _next(self):
        self._k, sub = jax.random.split(self._k)
        return sub
    def normal(self, shape):
        return jax.random.normal(self._next(), shape, dtype=jnp.bfloat16)
    def randint(self, lo, hi, shape):
        return jax.random.randint(self._next(), shape, lo, hi, dtype=jnp.int32)
    def uniform(self, shape, lo=0.0, hi=1.0):
        return jax.random.uniform(self._next(), shape, jnp.bfloat16, lo, hi)
    def permutation(self, n):
        return jax.random.permutation(self._next(), n)


kernel_name = 'standalone__sliding_block_cached__sampling'

def setup_inputs():
    _rng = _Rng(jax.random.key(int.from_bytes(__import__("os").urandom(4), "little")))
    _w = (lambda a: (lambda t: t.astype(jnp.bfloat16) if jnp.issubdtype(t.dtype, jnp.floating) else t)(jnp.asarray(a)))
    B, Sq, D = 8, 4, 640
    Hq, Hkv, Sk, Dh = 32, 32, 4096, 192
    assert Hq % Hkv == 0, (Hq, Hkv)
    return {
        "x": _w((lambda *s: _rng.normal(s) * 0.8)(B, Sq, D)),
        "k_cache": _w((lambda *s: _rng.normal(s) * 0.8)(B, Hkv, Sk, Dh)),
        "v_cache": _w((lambda *s: _rng.normal(s) * 0.05)(B, Hkv, Sk, Dh)),
        "wq": _w((lambda *s: _rng.normal(s) * 0.8)(D, Hq * Dh) * (D ** -0.5)),
        "wo": _w((lambda *s: _rng.normal(s) * 0.05)(Hq * Dh, D) * ((Hq * Dh) ** -0.5)),
    }

def reference(x, k_cache, v_cache, wq, wo):
    B, Sq, D = x.shape
    Hq, Dh = 32, 192
    Hkv, Sk = k_cache.shape[1], k_cache.shape[2]
    W = min(4096, max(256, Sk // 4))
    rep = Hq // Hkv
    q = (lambda x, *d: x.transpose(*d))((x @ wq).reshape(B, Sq, Hq, Dh), 0, 2, 1, 3)
    k = jnp.repeat(k_cache[:, :, Sk - W:, :], rep, axis=1)
    v = jnp.repeat(v_cache[:, :, Sk - W:, :], rep, axis=1)
    scores = jnp.einsum("bhqd,bhkd->bhqk", q, k) * (Dh ** -0.5)
    p = _softmax(scores, axis=-1)
    o = jnp.einsum("bhqk,bhkd->bhqd", p, v)
    return (lambda x, *d: x.transpose(*d))(o, 0, 2, 1, 3).reshape(B, Sq, Hq * Dh) @ wo
```

```python
import jax
import jax.numpy as jnp
from jax import lax
import jax.experimental.pallas as pl
import jax.experimental.pallas.tpu as pltpu

_NBUF = 4
_VSHIFT = 3


@jax.jit
def pallas_standalone__sliding_block_cached__sampling_kernel(
    x: jax.Array,
    k_cache: jax.Array,
    v_cache: jax.Array,
    wq: jax.Array,
    wo: jax.Array,
):
    B, SQ, D = x.shape
    H, DH = 32, 192
    Sk = k_cache.shape[2]
    W = min(4096, max(256, Sk // 4))
    NP = H // 2
    PD = 2 * DH
    NC = NP * B
    G = PD // 64
    NJ = W // 128
    scale = DH ** -0.5
    nbuf = _NBUF

    def kernel(x_hbm, kt_hbm, vt_hbm, wq_hbm, wo_hbm, o_ref,
               xbuf, kv, wqb, wob, x2, q2, ob, kvsem, wqsem, wosem, xsem):
        def kv_start(c):
            pair, b = c // B, c % B
            slot = c % nbuf
            blk = b * NP + pair
            for g in range(G):
                for s in range(2):
                    src = kt_hbm if s == 0 else vt_hbm
                    rows = pl.ds(((g + s * _VSHIFT) % G) * 64, 64)
                    for j in range(NJ):
                        pltpu.make_async_copy(
                            src.at[blk, rows, pl.ds(Sk - W + j * 128, 128)],
                            kv.at[slot, s, rows, pl.ds(j * 128, 128)],
                            kvsem.at[slot]).start(priority=j % 2)

        xc = pltpu.make_async_copy(x_hbm, xbuf, xsem)
        xc.start()

        def wq_start(jj, _):
            for g in range(D // 64):
                for q in range(2):
                    rows = pl.ds(g * 64, 64)
                    cols = pl.ds(pl.multiple_of((2 * jj + q) * 128, 128), 128)
                    pltpu.make_async_copy(
                        wq_hbm.at[rows, cols], wqb.at[rows, cols], wqsem).start(priority=q)
        lax.fori_loop(0, H * DH // 256, wq_start, None)
        lax.fori_loop(0, nbuf, lambda c, _: kv_start(c), None)

        xc.wait()
        for b in range(B):
            xb = xbuf[b].astype(jnp.float32)
            x2[pl.ds(8 * b, 4), :] = xb
            x2[pl.ds(8 * b + 4, 4), :] = xb
        pltpu.make_async_copy(wqb, wqb, wqsem).wait()

        def blockdiag(shape):
            r = lax.broadcasted_iota(jnp.int32, shape, 0)
            c = lax.broadcasted_iota(jnp.int32, shape, 1)
            return ((r % 8) < SQ) == (c < DH)

        def wo_start(p, _):
            for g in range(G):
                rows = pl.ds(g * 64, 64)
                pltpu.make_async_copy(
                    wo_hbm.at[p, rows], wob.at[p, rows], wosem.at[p]).start(priority=g % 2)

        def pair_body(pair, _):
            cols = pl.ds(pl.multiple_of(pair * PD, 128), PD)
            q = jnp.dot(x2[...].astype(jnp.bfloat16), wqb[:, cols],
                        preferred_element_type=jnp.float32)
            q2[...] = jnp.where(blockdiag(q.shape), q, 0.0)

            def b_body(b, _):
                c = pair * B + b
                slot = c % nbuf
                rows = pl.ds(pl.multiple_of(b * 8, 8), 8)
                qb = q2[rows, :].astype(jnp.bfloat16)
                pltpu.make_async_copy(kv.at[slot], kv.at[slot], kvsem.at[slot]).wait()
                s = jnp.dot(qb, kv[slot, 0], preferred_element_type=jnp.float32)
                m = jnp.max(s, axis=1, keepdims=True)
                p = jnp.exp((s - m) * scale)
                l = jnp.sum(p, axis=1, keepdims=True)
                o = lax.dot_general(p.astype(jnp.bfloat16), kv[slot, 1],
                                    (((1,), (1,)), ((), ())),
                                    preferred_element_type=jnp.float32)
                o = o / l
                ob[pair, rows, :] = jnp.where(blockdiag(o.shape), o, 0.0)

                @pl.when(c + nbuf < NC)
                def _():
                    kv_start(c + nbuf)

                @pl.when(c + nbuf == NC)
                def _():
                    lax.fori_loop(0, NP, wo_start, None)

            lax.fori_loop(0, B, b_body, None)

        lax.fori_loop(0, NP, pair_body, None)

        def proj(p, acc):
            pltpu.make_async_copy(wob.at[p], wob.at[p], wosem.at[p]).wait()
            return acc + jnp.dot(ob[p].astype(jnp.bfloat16), wob[p],
                                 preferred_element_type=jnp.float32)
        acc = lax.fori_loop(0, NP, proj, jnp.zeros((B * 8, D), jnp.float32))
        for b in range(B):
            o_ref[b] = (acc[8 * b:8 * b + 4, :] + acc[8 * b + 4:8 * b + 8, :]).astype(o_ref.dtype)

    kt = jnp.swapaxes(k_cache, 2, 3).reshape(B * NP, PD, Sk)
    vt = jnp.swapaxes(v_cache, 2, 3).reshape(B * NP, PD, Sk)
    wo3 = wo.reshape(NP, PD, D)
    return pl.pallas_call(
        kernel,
        out_shape=jax.ShapeDtypeStruct((B, SQ, D), x.dtype),
        in_specs=[pl.BlockSpec(memory_space=pl.ANY)] * 5,
        out_specs=pl.BlockSpec(memory_space=pltpu.VMEM),
        scratch_shapes=[
            pltpu.VMEM((B, SQ, D), jnp.bfloat16),
            pltpu.VMEM((nbuf, 2, PD, W), jnp.bfloat16),
            pltpu.VMEM((D, H * DH), jnp.bfloat16),
            pltpu.VMEM((NP, PD, D), jnp.bfloat16),
            pltpu.VMEM((B * 8, D), jnp.float32),
            pltpu.VMEM((B * 8, PD), jnp.float32),
            pltpu.VMEM((NP, B * 8, PD), jnp.float32),
            pltpu.SemaphoreType.DMA((nbuf,)),
            pltpu.SemaphoreType.DMA(()),
            pltpu.SemaphoreType.DMA((NP,)),
            pltpu.SemaphoreType.DMA(()),
        ],
        compiler_params=pltpu.CompilerParams(
            vmem_limit_bytes=64 * 1024 * 1024, disable_bounds_checks=True),
    )(x, kt, vt, wq, wo3)
```

```python
import jax
import jax.numpy as jnp
from jax import lax
import jax.experimental.pallas as pl
import jax.experimental.pallas.tpu as pltpu

_HQ, _DH = 32, 192
_NBUF = 4
_RG = 64
_LANES = 128


@jax.jit
def pallas_standalone__sliding_block_cached__sampling_kernel(
    x: jax.Array,
    k_cache: jax.Array,
    v_cache: jax.Array,
    wq: jax.Array,
    wo: jax.Array,
):
    B, SQ, D = x.shape
    Hkv, Sk = k_cache.shape[1], k_cache.shape[2]
    W = min(4096, max(256, Sk // 4))
    HD = _HQ * _DH
    NP = _HQ // 2
    PD = 2 * _DH
    NC = NP * B
    scale = _DH ** -0.5
    assert Hkv == _HQ and 2 * SQ == 8 and B % 2 == 0
    assert W % _LANES == 0 and (Sk - W) % _LANES == 0 and D % _RG == 0

    def kernel(x_hbm, kt_hbm, vt_hbm, wq_hbm, wo_hbm, o_ref,
               xbuf, kv, wqb, wob, x2, qq, ob, kvsem, wqsem, wosem, xsem):

        def kv_start(c):
            pair, b = c // B, c % B
            slot = c % _NBUF
            blk = b * NP + pair
            for g in range(PD // _RG):
                rows = pl.ds(g * _RG, _RG)
                for s, src in enumerate((kt_hbm, vt_hbm)):
                    for j in range(W // _LANES):
                        pltpu.make_async_copy(
                            src.at[blk, rows, pl.ds(Sk - W + j * _LANES, _LANES)],
                            kv.at[slot, s, rows, pl.ds(j * _LANES, _LANES)],
                            kvsem.at[slot],
                        ).start(priority=(j + s) % 2)

        def wq_start(jj, _):
            for g in range(D // _RG):
                rows = pl.ds(g * _RG, _RG)
                for j in range(2):
                    cols = pl.ds(pl.multiple_of((2 * jj + j) * _LANES, _LANES), _LANES)
                    pltpu.make_async_copy(
                        wq_hbm.at[rows, cols], wqb.at[rows, cols], wqsem
                    ).start(priority=j)

        def wo_start(pair, _):
            for g in range(PD // _RG):
                rows = pl.ds(g * _RG, _RG)
                pltpu.make_async_copy(
                    wo_hbm.at[pair, rows], wob.at[pair, rows], wosem.at[pair]
                ).start(priority=g % 2)

        def wait_filled(buf, sem):
            pltpu.make_async_copy(buf, buf, sem).wait()

        def first_head(shape):
            return lax.broadcasted_iota(jnp.int32, shape, 0) % 8 < SQ

        x_copy = pltpu.make_async_copy(x_hbm, xbuf, xsem)
        x_copy.start()
        lax.fori_loop(0, HD // (2 * _LANES), wq_start, None)
        lax.fori_loop(0, _NBUF, lambda c, _: kv_start(c), None)

        x_copy.wait()
        for b in range(B):
            xb = xbuf[b].astype(jnp.float32)
            x2[pl.ds(8 * b, SQ), :] = xb
            x2[pl.ds(8 * b + SQ, SQ), :] = xb
        wait_filled(wqb, wqsem)

        def attend(c, _):
            pair, b = c // B, c % B
            slot = c % _NBUF
            cols = pl.ds(pl.multiple_of(pair * PD, _LANES), PD)
            rows = pl.ds(pl.multiple_of(b * 8, 8), 8)

            @pl.when(b == 0)
            def _():
                q = jnp.dot(x2[...].astype(wqb.dtype), wqb[:, cols],
                            preferred_element_type=jnp.float32)
                qq[...] = jnp.where(first_head((8 * B, _DH)), q[:, :_DH], q[:, _DH:])

            qb = qq[rows, :].astype(kv.dtype)
            wait_filled(kv.at[slot], kvsem.at[slot])
            s0 = jnp.dot(qb, kv[slot, 0, :_DH], preferred_element_type=jnp.float32)
            s1 = jnp.dot(qb, kv[slot, 0, _DH:], preferred_element_type=jnp.float32)
            s = jnp.where(first_head(s0.shape), s0, s1)
            m = jnp.max(s, axis=1, keepdims=True)
            p = jnp.exp((s - m) * scale)
            l = jnp.sum(p, axis=1, keepdims=True)
            o = lax.dot_general(p.astype(kv.dtype), kv[slot, 1], (((1,), (1,)), ((), ())),
                                preferred_element_type=jnp.float32) / l
            own = first_head(o.shape) == (lax.broadcasted_iota(jnp.int32, o.shape, 1) < _DH)
            ob[rows, cols] = jnp.where(own, o, 0.0)

            @pl.when(c + _NBUF < NC)
            def _():
                kv_start(c + _NBUF)

            @pl.when(c + _NBUF == NC)
            def _():
                lax.fori_loop(0, NP, wo_start, None)

        lax.fori_loop(0, NC, attend, None)

        def project(pair, acc):
            o = ob[:, pl.ds(pl.multiple_of(pair * PD, _LANES), PD)].reshape(B // 2, 2, 8, PD)
            even, odd = o[:, 0], o[:, 1]
            even = even + pltpu.roll(even, SQ, 1)
            odd = odd + pltpu.roll(odd, SQ, 1)
            r = lax.broadcasted_iota(jnp.int32, even.shape, 1)
            lhs = jnp.where(r < SQ, even, odd).reshape(B * SQ, PD).astype(wob.dtype)
            wait_filled(wob.at[pair], wosem.at[pair])
            return acc + jnp.dot(lhs, wob[pair], preferred_element_type=jnp.float32)

        acc = lax.fori_loop(0, NP, project, jnp.zeros((B * SQ, D), jnp.float32))
        for b in range(B):
            o_ref[b] = acc[SQ * b:SQ * (b + 1), :].astype(o_ref.dtype)

    kt = jnp.swapaxes(k_cache, 2, 3).reshape(B * NP, PD, Sk)
    vt = jnp.swapaxes(v_cache, 2, 3).reshape(B * NP, PD, Sk)
    return pl.pallas_call(
        kernel,
        out_shape=jax.ShapeDtypeStruct((B, SQ, D), x.dtype),
        in_specs=[pl.BlockSpec(memory_space=pl.ANY)] * 5,
        out_specs=pl.BlockSpec(memory_space=pltpu.VMEM),
        scratch_shapes=[
            pltpu.VMEM((B, SQ, D), x.dtype),
            pltpu.VMEM((_NBUF, 2, PD, W), k_cache.dtype),
            pltpu.VMEM((D, HD), wq.dtype),
            pltpu.VMEM((NP, PD, D), wo.dtype),
            pltpu.VMEM((B * 8, D), jnp.float32),
            pltpu.VMEM((B * 8, _DH), jnp.float32),
            pltpu.VMEM((B * 8, HD), jnp.float32),
            pltpu.SemaphoreType.DMA((_NBUF,)),
            pltpu.SemaphoreType.DMA(()),
            pltpu.SemaphoreType.DMA((NP,)),
            pltpu.SemaphoreType.DMA(()),
        ],
        compiler_params=pltpu.CompilerParams(vmem_limit_bytes=48 * 1024 * 1024),
    )(x, kt, vt, wq, wo.reshape(NP, PD, D))
```
